```python
import os as _os
_os.environ.setdefault("JAX_PLATFORMS", "cpu")
import jax
import jax.numpy as jnp

def _softmax(x, axis=-1):
    return jax.nn.softmax(x, axis=axis)
def _gelu(x):
    return jax.nn.gelu(x, approximate=True)
def _silu(x):
    return jax.nn.silu(x)
def _sigmoid(x):
    return jax.nn.sigmoid(x)
def _layernorm(x, axis=-1, eps=1e-5):
    m = jnp.mean(x, axis=axis, keepdims=True)
    v = jnp.var(x, axis=axis, keepdims=True)
    return (x - m) / jnp.sqrt(v + eps)
def _scatter_add(tgt, idx, src, axis=0):
    return tgt.at[idx].add(src)
def _segment_sum(src, seg, n):
    return jax.ops.segment_sum(src, seg, n)
class _Rng:
    def __init__(self, key):
        self._k = key
    def _next(self):
        self._k, sub = jax.random.split(self._k)
        return sub
    def normal(self, shape):
        return jax.random.normal(self._next(), shape, dtype=jnp.bfloat16)
    def randint(self, lo, hi, shape):
        return jax.random.randint(self._next(), shape, lo, hi, dtype=jnp.int32)
    def uniform(self, shape, lo=0.0, hi=1.0):
        return jax.random.uniform(self._next(), shape, jnp.bfloat16, lo, hi)
    def permutation(self, n):
        return jax.random.permutation(self._next(), n)


kernel_name = 'parallel_sum__softmax_full_mha__moe_arch_mod__prompt'

def setup_inputs():
    _rng = _Rng(jax.random.key(int.from_bytes(__import__("os").urandom(4), "little")))
    _w = (lambda a: (lambda t: t.astype(jnp.bfloat16) if jnp.issubdtype(t.dtype, jnp.floating) else t)(jnp.asarray(a)))
    def _A_setup():
        B, S, D = 1, 2048, 512
        return {
            "x": _w((lambda *s: _rng.normal(s) * 0.05)(B, S, D)),
            "wqkv": _w((lambda *s: _rng.normal(s) * 0.1)(D, 3 * D)),
            "wo": _w((lambda *s: _rng.normal(s) * 0.05)(D, D)),
        }
    _A_in = _A_setup()

    def _B_setup():
        B, S, D, F, C = 1, 2048, 512, 1792, 1
        return {
            "x": _w((lambda *s: _rng.normal(s) * 0.05)(B, S, D)),
            "w_r": _w((lambda *s: _rng.normal(s) * 1.6)(D)),
            "w_gate": _w((lambda *s: _rng.normal(s) * 0.1)(D, F)),
            "w_up": _w((lambda *s: _rng.normal(s) * 0.1)(D, F)),
            "w_down": _w((lambda *s: _rng.normal(s) * 0.1)(F, D)),
        }
    _B_in = _B_setup()

    return {
        "A_x": _A_in["x"],
        "A_wqkv": _A_in["wqkv"],
        "A_wo": _A_in["wo"],
        "B_x": _B_in["x"],
        "B_w_r": _B_in["w_r"],
        "B_w_gate": _B_in["w_gate"],
        "B_w_up": _B_in["w_up"],
        "B_w_down": _B_in["w_down"],
    }

def reference(A_x, A_wqkv, A_wo, B_x, B_w_r, B_w_gate, B_w_up, B_w_down):
    def _A_ref(x, wqkv, wo):
        B, S, D = x.shape
        H = 32; Dh = D // H
        qkv = (lambda x, *d: x.transpose(*d))((x @ wqkv).reshape(B, S, 3, H, Dh), 2, 0, 3, 1, 4)
        q, k, v = qkv[0], qkv[1], qkv[2]
        scale = Dh ** -0.5
        scores = jnp.einsum("bhqd,bhkd->bhqk", q, k) * scale
        p = _softmax(scores, axis=-1)
        o = jnp.einsum("bhqk,bhkd->bhqd", p, v)
        return (lambda x, *d: x.transpose(*d))(o, 0, 2, 1, 3).reshape(B, S, D) @ wo

    def _B_ref(x, w_r, w_gate, w_up, w_down):
        B, S, D = x.shape
        C = 1
        r = x @ w_r
        idx = jnp.argsort(-r, axis=-1)[:, :C]
        idx_e = jnp.repeat(idx.reshape(B, C, 1), D, axis=2)
        x_sel = jnp.take_along_axis(x, idx_e, axis=1)
        g = _silu(x_sel @ w_gate)
        u = x_sel @ w_up
        y = (g * u) @ w_down
        r_sel = _sigmoid(jnp.take_along_axis(r, idx, axis=1))
        y = y * r_sel.reshape(B, C, 1)
        b_off = (jnp.arange(B) * S).reshape(B, 1)
        flat_idx = (idx + b_off).reshape(B * C)
        zero = (x * 0.0).reshape(B * S, D)
        upd = _scatter_add(zero, flat_idx, y.reshape(B * C, D), axis=0)
        return x + upd.reshape(B, S, D)

    x = A_x
    xn = _layernorm(x, axis=-1)
    return x + _A_ref(xn, A_wqkv, A_wo) + _B_ref(xn, B_w_r, B_w_gate, B_w_up, B_w_down)
```

```python
import functools
import math

import jax
import jax.numpy as jnp
import jax.experimental.pallas as pl
import jax.experimental.pallas.tpu as pltpu

_H = 32
_EPS = 1e-5
_LOG2E = math.log2(math.e)

_NT = (((1,), (1,)), ((), ()))


def _bf16_round(v):
    return v.astype(jnp.bfloat16).astype(jnp.float32)


def _kernel(x_hbm, wqkv_hbm, wo_hbm, wr_hbm, wg_hbm, wu_hbm, wd_hbm,
            o_hbm,
            x_ref, wqkv_ref, wt_ref, wo_ref, o_ref,
            xn_ref, k_ref, qt_ref, vt_ref, s_ref, m_ref, ot_ref, part_ref, r_ref,
            wg_ref, wu_ref, wd_ref, wr_ref, sems, xsems, osems,
            *, S, D, F, TQ, TK, TC, G):
    H = _H
    Dh = D // H
    NQ = S // TQ
    NKC = S // TK
    NC = S // TC
    f32 = jnp.float32
    bf16 = jnp.bfloat16

    xparts = [(0, TC), (TC, 2 * TC)] + [(lo, lo + 2 * TC) for lo in range(2 * TC, S, 2 * TC)]

    def x_copy(i):
        lo, hi = xparts[i]
        return pltpu.make_async_copy(x_hbm.at[lo:hi, :], x_ref.at[lo:hi, :], xsems.at[i])

    def w_copy(j):
        return pltpu.make_async_copy(wqkv_hbm.at[:, j * D:(j + 1) * D], wqkv_ref.at[j],
                                     sems.at[3 + j])

    cp_o = pltpu.make_async_copy(wo_hbm, wo_ref, sems.at[6])
    cp_r = pltpu.make_async_copy(wr_hbm, wr_ref.at[0:D], sems.at[7])
    cp_g = pltpu.make_async_copy(wg_hbm, wg_ref, sems.at[0])
    cp_u = pltpu.make_async_copy(wu_hbm, wu_ref, sems.at[1])
    cp_d = pltpu.make_async_copy(wd_hbm, wd_ref, sems.at[2])
    x_copy(0).start()
    w_copy(1).start()
    cp_r.start()
    x_copy(1).start()
    w_copy(0).start()
    w_copy(2).start()

    def layernorm(i):
        x = x_ref[i * TC:(i + 1) * TC, :].astype(f32)
        mean = jnp.mean(x, axis=-1, keepdims=True)
        cen = x - mean
        var = jnp.mean(cen * cen, axis=-1, keepdims=True)
        m_b = _bf16_round(mean)
        v_b = _bf16_round(var)
        den = _bf16_round(jnp.sqrt(_bf16_round(v_b + _EPS)))
        num = _bf16_round(x - m_b)
        xn_ref[i * TC:(i + 1) * TC, :] = (num * (1.0 / den)).astype(bf16)

    x_copy(0).wait()
    for j in range(2, len(xparts)):
        x_copy(j).start()
    layernorm(0)

    qscale = (Dh ** -0.5) * _LOG2E

    def k_proj(i):
        xn = xn_ref[i * TC:(i + 1) * TC, :]
        kk = jnp.dot(xn, wqkv_ref[1], preferred_element_type=f32)
        for j in range(H // G):
            slab, off = divmod(j * G * Dh, 128)
            kj = kk[:, slab * 128:(slab + 1) * 128]
            if off:
                kj = pltpu.roll(kj, 128 - off, 1)
            k_ref[j, i * TC:(i + 1) * TC, :] = kj.astype(bf16)

    def qv_proj(i):
        xn = xn_ref[i * TC:(i + 1) * TC, :]
        qt = jax.lax.dot_general(wt_ref[0], xn, _NT, preferred_element_type=f32)
        qt = (_bf16_round(qt) * qscale).astype(bf16)
        vt = jax.lax.dot_general(wt_ref[1], xn, _NT, preferred_element_type=f32).astype(bf16)
        rt = jax.lax.dot_general(wr8, xn, _NT, preferred_element_type=f32)
        r_ref[:, i * TC:(i + 1) * TC] = rt
        qb, qo = divmod(i * TC, TQ)
        for h in range(H):
            qt_ref[qb, h, :, qo:qo + TC] = qt[h * Dh:(h + 1) * Dh, :]
            for j in range(TC // 128):
                kc, ko = divmod(i * TC + j * 128, TK)
                vt_ref[h, kc, :, ko:ko + 128] = vt[h * Dh:(h + 1) * Dh, j * 128:(j + 1) * 128]

    w_copy(1).wait()
    cp_r.wait()
    wr8 = jnp.broadcast_to(wr_ref[0:D].reshape(1, D), (8, D))
    k_proj(0)
    w_copy(0).wait()
    w_copy(2).wait()
    x_copy(1).wait()
    cp_o.start()
    layernorm(1)
    wt_ref[0] = wqkv_ref[0].astype(f32).T.astype(bf16)
    wt_ref[1] = wqkv_ref[2].astype(f32).T.astype(bf16)
    k_proj(1)
    for i in range(NC):
        if i + 2 < NC:
            if i % 2 == 0:
                x_copy(2 + i // 2).wait()
                if i == 0:
                    cp_g.start()
                    cp_u.start()
                    cp_d.start()
                if i == 2:
                    cp_o.wait()
                    wt_ref[2] = wo_ref[...].astype(f32).T.astype(bf16)
            layernorm(i + 2)
        qv_proj(i)
        if i + 2 < NC:
            k_proj(i + 2)

    def routed_ffn():
        r = _bf16_round(r_ref[...])
        rmax = jnp.max(r, axis=-1, keepdims=True)
        lane = jax.lax.broadcasted_iota(jnp.int32, (8, S), 1)
        idx = jnp.min(jnp.where(r == rmax, lane, S), axis=-1, keepdims=True)
        idx = jnp.minimum(idx, S - 1)
        i0 = jnp.min(idx)
        rb = pl.multiple_of(jax.lax.shift_right_logical(i0, 4) * 16, 16)
        blk = xn_ref[pl.ds(rb, 16), :].astype(f32)
        sel = (jax.lax.broadcasted_iota(jnp.int32, (16, D), 0) + rb) == i0
        x_row = jnp.sum(jnp.where(sel, blk, 0.0), axis=0, keepdims=True)
        x_sel = jnp.broadcast_to(x_row, (8, D)).astype(bf16)
        yield
        hs = []
        for j in range(F // 128):
            gpre = _bf16_round(jnp.dot(x_sel, wg_ref[:, j * 128:(j + 1) * 128],
                                       preferred_element_type=f32))
            yield
            u = _bf16_round(jnp.dot(x_sel, wu_ref[:, j * 128:(j + 1) * 128],
                                    preferred_element_type=f32))
            g = _bf16_round(gpre * jax.nn.sigmoid(gpre))
            hs.append((g * u).astype(bf16))
            yield
        y = None
        for j in range(F // 128):
            t = jnp.dot(hs[j], wd_ref[j * 128:(j + 1) * 128, :], preferred_element_type=f32)
            y = t if y is None else y + t
            yield
        y = _bf16_round(_bf16_round(y) * _bf16_round(jax.nn.sigmoid(rmax)))
        y16 = jnp.concatenate([y, y], axis=0)
        xn_ref[pl.ds(rb, 16), :] = (blk + jnp.where(sel, y16, 0.0)).astype(bf16)

    nb = NQ * H
    nit = nb // G
    LOG2H = H.bit_length() - 1
    LOG2G = G.bit_length() - 1

    def split(b):
        if isinstance(b, int):
            return b // H, b % H
        return jax.lax.shift_right_logical(b, LOG2H), jnp.bitwise_and(b, H - 1)

    def col_max8(sc):
        return sc.reshape(TK // 8, 8, TQ).max(axis=0)

    def col_sum8(p):
        tot = None
        for t in range(TK // 128):
            for j in reversed(range(8)):
                r0 = t * 128 + j * 16
                pair = p[r0:r0 + 8, :] + p[r0 + 8:r0 + 16, :]
                tot = pair if tot is None else tot + pair
        return tot

    neg = jnp.full((8, TQ), -jnp.inf, f32)

    def masked_q(qb, h, g):
        parts = []
        if g > 0:
            parts.append(jnp.zeros((g * Dh, TQ), bf16))
        parts.append(qt_ref[qb, h])
        if (g + 1) * Dh < 128:
            parts.append(jnp.zeros((128 - (g + 1) * Dh, TQ), bf16))
        return jnp.concatenate(parts, axis=0)

    def qk_chunk(qb, h, c, g, mrun):
        kg = h // G if isinstance(h, int) else jax.lax.shift_right_logical(h, LOG2G)
        kblk = k_ref[kg, c * TK:(c + 1) * TK, :]
        sc = jnp.dot(kblk, masked_q(qb, h, g), preferred_element_type=f32)
        s_ref[g, c * TK:(c + 1) * TK, :] = sc
        return jnp.maximum(mrun, col_max8(sc))

    def store_max(g, mrun):
        m_ref[g] = jnp.broadcast_to(jnp.max(mrun, axis=0, keepdims=True), (8, TQ))

    cp_g.wait()
    cp_u.wait()
    cp_d.wait()
    ffn = routed_ffn()
    npieces = 3 * (F // 128) + 2
    done = 0
    for g in range(G):
        mrun = neg
        for c in range(NKC):
            mrun = qk_chunk(0, g, c, g, mrun)
            want = ((g * NKC + c + 1) * npieces + G * NKC - 1) // (G * NKC)
            while done < want:
                next(ffn, None)
                done += 1
        store_max(g, mrun)
    for _ in ffn:
        pass

    KL = (H - G) * Dh // 128 * 128

    def out_partial(n, r):
        c0 = r * 128
        part_ref[n, r] = jnp.dot(wt_ref[2, c0:c0 + 128, 0:KL],
                                 ot_ref[NQ - 1, 0:KL, n * 128:(n + 1) * 128],
                                 preferred_element_type=f32)

    def out_piece(qb, n, r):
        r0 = qb * TQ + n * 128
        c0 = r * 128
        if qb == NQ - 1:
            att_t = part_ref[n, r] + jnp.dot(wt_ref[2, c0:c0 + 128, KL:D],
                                             ot_ref[qb, KL:D, n * 128:(n + 1) * 128],
                                             preferred_element_type=f32)
        else:
            att_t = jnp.dot(wt_ref[2, c0:c0 + 128, :], ot_ref[qb, :, n * 128:(n + 1) * 128],
                            preferred_element_type=f32)
        att = att_t.T
        x = x_ref[r0:r0 + 128, c0:c0 + 128].astype(f32)
        xn = xn_ref[r0:r0 + 128, c0:c0 + 128].astype(f32)
        res = _bf16_round(x + _bf16_round(att)) + xn
        o_ref[r0:r0 + 128, c0:c0 + 128] = res.astype(o_ref.dtype)

    oparts = [(qb * TQ, (qb + 1) * TQ) for qb in range(NQ - 1)]
    oparts += [((NQ - 1) * TQ + n * 128, (NQ - 1) * TQ + (n + 1) * 128) for n in range(TQ // 128)]

    def out_copy(j):
        lo, hi = oparts[j]
        return pltpu.make_async_copy(o_ref.at[lo:hi, :], o_hbm.at[lo:hi, :], osems.at[j])

    def group(it, last):
        pieces = [(qb, n, r) for qb in range(NQ) for n in range(TQ // 128)
                  for r in range(D // 128)] if last else []
        nslots = G * NKC
        for g in range(G):
            qb, h = split(it * G + g)
            if not last:
                qbn, hn = split((it + 1) * G + g)
            m_cur = m_ref[g]
            mrun = neg
            lsum = jnp.zeros((8, TQ), f32)
            acc = jnp.zeros((Dh, TQ), f32)
            for c in range(NKC):
                sc = s_ref[g, c * TK:(c + 1) * TK, :]
                p = jnp.exp2((sc.reshape(TK // 8, 8, TQ) - m_cur[None]).reshape(TK, TQ))
                if not last:
                    mrun = qk_chunk(qbn, hn, c, g, mrun)
                else:
                    slot = g * NKC + c
                    lo = slot * len(pieces) // nslots
                    hi = (slot + 1) * len(pieces) // nslots
                    for (pq, pn, pr) in pieces[lo:hi]:
                        if pq == NQ - 1:
                            out_partial(pn, pr)
                            continue
                        out_piece(pq, pn, pr)
                        if pn == TQ // 128 - 1 and pr == D // 128 - 1:
                            out_copy(pq).start()
                lsum = lsum + col_sum8(p)
                acc = acc + jnp.dot(vt_ref[h, c], p.astype(bf16), preferred_element_type=f32)
            if not last:
                store_max(g, mrun)
            l = jnp.sum(lsum, axis=0, keepdims=True)
            orow = h * Dh if isinstance(h, int) else pl.multiple_of(h * Dh, Dh)
            ot_ref[qb, pl.ds(orow, Dh), :] = (acc / l).astype(bf16)

    def iter_body(it, carry):
        group(it, False)
        return carry

    jax.lax.fori_loop(0, nit - 1, iter_body, 0)

    group(nit - 1, True)
    for n in range(TQ // 128):
        for r in range(D // 128):
            out_piece(NQ - 1, n, r)
        out_copy(NQ - 1 + n).start()
    for j in range(len(oparts)):
        out_copy(j).wait()


@functools.partial(jax.jit, static_argnames=("TQ", "TK", "G", "TC"))
def _forward(A_x, A_wqkv, A_wo, B_w_r, B_w_gate, B_w_up, B_w_down,
             TQ=512, TK=128, G=4, TC=256):
    B, S, D = A_x.shape
    assert B == 1
    F = B_w_gate.shape[1]
    H = _H
    Dh = D // H
    x2 = A_x.reshape(S, D)
    bf16 = jnp.bfloat16
    f32 = jnp.float32

    kern = functools.partial(_kernel, S=S, D=D, F=F, TQ=TQ, TK=TK, TC=TC, G=G)
    hbm = pl.BlockSpec(memory_space=pl.ANY)
    out = pl.pallas_call(
        kern,
        out_shape=jax.ShapeDtypeStruct((S, D), A_x.dtype),
        in_specs=[hbm] * 7,
        out_specs=hbm,
        scratch_shapes=[
            pltpu.VMEM((S, D), bf16),
            pltpu.VMEM((3, D, D), bf16),
            pltpu.VMEM((3, D, D), bf16),
            pltpu.VMEM((D, D), bf16),
            pltpu.VMEM((S, D), bf16),
            pltpu.VMEM((S, D), bf16),
            pltpu.VMEM((H // G, S, 128), bf16),
            pltpu.VMEM((S // TQ, H, Dh, TQ), bf16),
            pltpu.VMEM((H, S // TK, Dh, TK), bf16),
            pltpu.VMEM((G, S, TQ), f32),
            pltpu.VMEM((G, 8, TQ), f32),
            pltpu.VMEM((S // TQ, D, TQ), bf16),
            pltpu.VMEM((TQ // 128, D // 128, 128, 128), f32),
            pltpu.VMEM((8, S), f32),
            pltpu.VMEM((D, F), bf16),
            pltpu.VMEM((D, F), bf16),
            pltpu.VMEM((F, D), bf16),
            pltpu.VMEM((max(D, 2048),), bf16),
            pltpu.SemaphoreType.DMA((8,)),
            pltpu.SemaphoreType.DMA((S // (2 * TC) + 1,)),
            pltpu.SemaphoreType.DMA((S // TQ - 1 + TQ // 128,)),
        ],
        compiler_params=pltpu.CompilerParams(vmem_limit_bytes=100 * 1024 * 1024),
    )(x2, A_wqkv, A_wo, B_w_r, B_w_gate, B_w_up, B_w_down)
    return out.reshape(B, S, D)


@jax.jit
def pallas_parallel_sum__softmax_full_mha__moe_arch_mod__prompt_kernel(
    A_x: jax.Array,
    A_wqkv: jax.Array,
    A_wo: jax.Array,
    B_x: jax.Array,
    B_w_r: jax.Array,
    B_w_gate: jax.Array,
    B_w_up: jax.Array,
    B_w_down: jax.Array,
):
    del B_x
    return _forward(A_x, A_wqkv, A_wo, B_w_r, B_w_gate, B_w_up, B_w_down)
```
